```python
import os as _os
_os.environ.setdefault("JAX_PLATFORMS", "cpu")
import jax
import jax.numpy as jnp

def _softmax(x, axis=-1):
    return jax.nn.softmax(x, axis=axis)
def _gelu(x):
    return jax.nn.gelu(x, approximate=True)
def _silu(x):
    return jax.nn.silu(x)
def _sigmoid(x):
    return jax.nn.sigmoid(x)
def _layernorm(x, axis=-1, eps=1e-5):
    m = jnp.mean(x, axis=axis, keepdims=True)
    v = jnp.var(x, axis=axis, keepdims=True)
    return (x - m) / jnp.sqrt(v + eps)
def _scatter_add(tgt, idx, src, axis=0):
    return tgt.at[idx].add(src)
def _segment_sum(src, seg, n):
    return jax.ops.segment_sum(src, seg, n)
class _Rng:
    def __init__(self, key):
        self._k = key
    def _next(self):
        self._k, sub = jax.random.split(self._k)
        return sub
    def normal(self, shape):
        return jax.random.normal(self._next(), shape, dtype=jnp.bfloat16)
    def randint(self, lo, hi, shape):
        return jax.random.randint(self._next(), shape, lo, hi, dtype=jnp.int32)
    def uniform(self, shape, lo=0.0, hi=1.0):
        return jax.random.uniform(self._next(), shape, jnp.bfloat16, lo, hi)
    def permutation(self, n):
        return jax.random.permutation(self._next(), n)


kernel_name = 'concat_heads__gqa_block_cached__mha_block_cached__near_ridge'

def setup_inputs():
    _rng = _Rng(jax.random.key(int.from_bytes(__import__("os").urandom(4), "little")))
    _w = (lambda a: (lambda t: t.astype(jnp.bfloat16) if jnp.issubdtype(t.dtype, jnp.floating) else t)(jnp.asarray(a)))
    def _A_setup():
        B, Sq, D = 8, 224, 512
        Hq, Hkv, Sk, Dh = 32, 32, 512, 128
        assert Hq % Hkv == 0, (Hq, Hkv)
        return {
            "x": _w((lambda *s: _rng.normal(s) * 0.8)(B, Sq, D)),
            "k_cache": _w((lambda *s: _rng.normal(s) * 0.8)(B, Hkv, Sk, Dh)),
            "v_cache": _w((lambda *s: _rng.normal(s) * 0.05)(B, Hkv, Sk, Dh)),
            "wq": _w((lambda *s: _rng.normal(s) * 0.8)(D, Hq * Dh) * (D ** -0.5)),
            "wo": _w((lambda *s: _rng.normal(s) * 0.05)(Hq * Dh, D) * ((Hq * Dh) ** -0.5)),
        }
    _A_in = _A_setup()

    def _B_setup():
        B, Sq, D = 8, 224, 512
        H, Sk, Dh = 32, 512, 128
        return {
            "x": _w((lambda *s: _rng.normal(s) * 0.8)(B, Sq, D)),
            "k_cache": _w((lambda *s: _rng.normal(s) * 0.8)(B, H, Sk, Dh)),
            "v_cache": _w((lambda *s: _rng.normal(s) * 0.05)(B, H, Sk, Dh)),
            "wq": _w((lambda *s: _rng.normal(s) * 0.8)(D, H * Dh) * (D ** -0.5)),
            "wo": _w((lambda *s: _rng.normal(s) * 0.05)(H * Dh, D) * ((H * Dh) ** -0.5)),
        }
    _B_in = _B_setup()

    return {
        "A_x": _A_in["x"],
        "A_k_cache": _A_in["k_cache"],
        "A_v_cache": _A_in["v_cache"],
        "A_wq": _A_in["wq"],
        "A_wo": _A_in["wo"],
        "B_x": _B_in["x"],
        "B_k_cache": _B_in["k_cache"],
        "B_v_cache": _B_in["v_cache"],
        "B_wq": _B_in["wq"],
        "B_wo": _B_in["wo"],
    }

def reference(A_x, A_k_cache, A_v_cache, A_wq, A_wo, B_x, B_k_cache, B_v_cache, B_wq, B_wo):
    def _A_ref(x, k_cache, v_cache, wq, wo):
        B, Sq, D = x.shape
        Hq, Dh = 32, 128
        Hkv = k_cache.shape[1]
        rep = Hq // Hkv
        q = (lambda x, *d: x.transpose(*d))((x @ wq).reshape(B, Sq, Hq, Dh), 0, 2, 1, 3)
        k = jnp.repeat(k_cache, rep, axis=1)
        v = jnp.repeat(v_cache, rep, axis=1)
        scores = jnp.einsum("bhqd,bhkd->bhqk", q, k) * (Dh ** -0.5)
        p = _softmax(scores, axis=-1)
        o = jnp.einsum("bhqk,bhkd->bhqd", p, v)
        return (lambda x, *d: x.transpose(*d))(o, 0, 2, 1, 3).reshape(B, Sq, Hq * Dh) @ wo

    def _B_ref(x, k_cache, v_cache, wq, wo):
        B, Sq, D = x.shape
        H, Dh = 32, 128
        q = (lambda x, *d: x.transpose(*d))((x @ wq).reshape(B, Sq, H, Dh), 0, 2, 1, 3)
        scores = jnp.einsum("bhqd,bhkd->bhqk", q, k_cache) * (Dh ** -0.5)
        p = _softmax(scores, axis=-1)
        o = jnp.einsum("bhqk,bhkd->bhqd", p, v_cache)
        return (lambda x, *d: x.transpose(*d))(o, 0, 2, 1, 3).reshape(B, Sq, H * Dh) @ wo

    a = _A_ref(A_x, A_k_cache, A_v_cache, A_wq, A_wo)
    b = _B_ref(B_x, B_k_cache, B_v_cache, B_wq, B_wo)
    return jnp.concatenate([a, b], axis=-1)
```

```python
import functools
import jax
import jax.numpy as jnp
from jax import lax
import jax.experimental.pallas as pl
import jax.experimental.pallas.tpu as pltpu

LOG2E = 1.4426950408889634
F32, BF16, I32 = jnp.float32, jnp.bfloat16, jnp.int32
NB = 8
HW = 256
T = 7

def _mm(a, b):
    return jnp.dot(a.astype(BF16), b.astype(BF16), preferred_element_type=F32)

def _quads(m):
    r, c = m.shape[0] // 2, m.shape[1] // 2
    return m[:r, :c], m[:r, c:], m[r:, :c], m[r:, c:]

def _alpha(a11, a12, a21, a22):
    return [lambda: a11() + a22(), lambda: a21() + a22(), a11, a22, lambda: a11() + a12(), lambda: a21() - a11(), lambda: a12() - a22()]

def _beta(m):
    b11, b12, b21, b22 = _quads(m)
    return [b11 + b22, b11, b12 - b22, b21 - b11, b22, b11 + b12, b21 + b22]

def _gamma(m):
    return [(m[0] + m[6]) + (m[3] - m[4]), m[2] + m[4], m[1] + m[3], (m[0] + m[5]) + (m[2] - m[1])]

class Cfg:
    ahead = 3; glue = 1; only_l = False; newton = True; npairs = NB
    def __init__(self, **kw):
        for k, v in kw.items(): object.__setattr__(self, k, v)

def _kernel(xa, ka, va, wqa, woa, xb, kb, vb, wqb, wob, out,
            x_s, wq_s, wo_s, kv_s, xf, tf, sf, uf, rf, md_s, mu_s, gb_s, ga_s, accb, acca, ob_s, sem, sem_o, *, cfg):
    hbm = ((xa, ka, va, wqa, woa), (xb, kb, vb, wqb, wob))
    c = (128 ** -0.5) * LOG2E
    lo, hi = slice(0, HW), slice(HW, 2 * HW)
    f = lambda t: t.astype(F32)
    h = lambda t: t.astype(BF16)
    SQ = x_s.shape[2]; HR = SQ // 2
    top, bot = slice(0, HR), slice(HR, SQ)

    def w_copy(p, name, g, dst=None):
        x, k, v, wq, wo = hbm[p]
        d = p if dst is None else dst
        off = g * 512 if isinstance(g, int) else pl.multiple_of(g * 512, 512)
        s = sem.at[2 * NB + (d * 5 + "xutrs".index(name)) * NB + g]
        if name == "x": return pltpu.make_async_copy(x.at[g], x_s.at[d, g], s)
        if name == "u": return pltpu.make_async_copy(wq.at[:, pl.ds(off, HW)], wq_s.at[d, g, 0], s)
        if name == "t": return pltpu.make_async_copy(wq.at[:, pl.ds(off + HW, HW)], wq_s.at[d, g, 1], s)
        if name == "r": return pltpu.make_async_copy(wo.at[pl.ds(off, HW), :], wo_s.at[d, g, 0], s)
        if name == "s": return pltpu.make_async_copy(wo.at[pl.ds(off + HW, HW), :], wo_s.at[d, g, 1], s)

    def start_kv(p, a, j):
        x, k, v, wq, wo = hbm[p]
        b = (a + j + 1) % NB
        for n in (0, 2, 1, 3):
            src = (k, k, v, v)[n]
            src = src.at[a, b, 1] if n % 2 == 0 else src.at[b, a, 0]
            pltpu.make_async_copy(src, kv_s.at[a % 2, j, n], sem.at[(a % 2) * NB + j]).start()

    def start_first(j):
        b = (j + 1) % NB
        if j == 0:
            w_copy(0, "x", 0).start(); w_copy(0, "u", 0).start()
        if b: w_copy(0, "x", b).start()
        w_copy(0, "t", b).start()
        start_kv(0, 0, j)
        if j == 0: w_copy(0, "r", 0).start()
        w_copy(0, "s", b).start()
        if j == 5: w_copy(0, "u", 1).start()
        if j == 7: w_copy(0, "r", 1).start()

    def out_copy(part, b):
        col = part * 512 if isinstance(part, int) else pl.multiple_of(part * 512, 512)
        return pltpu.make_async_copy(ob_s.at[part, b], out.at[b, :, pl.ds(col, 512)], sem_o.at[part, b])

    def iteration(part, a, first, order):
        slot = a % 2
        bs = [(a + j + 1) % NB for j in range(NB)]
        an = bs[0]
        val = {}
        zero = jnp.full((8, 128), lax.shift_right_logical(part, 1), I32)
        def memo(key, fn):
            if key not in val: val[key] = fn()
            return val[key]
        def D(j):
            t = j + cfg.ahead
            if first and t < NB:
                pl.when(part == 0)(lambda: start_first(t))
                pl.when(part == 1)(lambda: start_kv(1, a, t))
            elif t < NB:
                for p in range(2): pl.when(part == p)(lambda: start_kv(p, a, t))
            elif first:
                for p in range(2): pl.when(part == p)(lambda: start_kv(p, an, t - NB))
            else:
                nxt = part + (a + 1) // NB
                for p in range(2): pl.when(nxt == p)(lambda: start_kv(p, an, t - NB))
            if first and j == NB - 1:
                @pl.when(part == 0)
                def _():
                    w_copy(0, "u", 2).start()
                    for n in "xutrs": w_copy(1, n, 0).start()
            if not first and j < 5:
                pl.when(part == 0)(lambda: w_copy(1, "xutrs"[j], a).start())
            if not first and j == 5:
                pl.when(jnp.logical_and(part == 0, a < NB - 1))(lambda: w_copy(0, "r", an).start())
            if not first and j == 6:
                pl.when(jnp.logical_and(part == 0, a < NB - 2))(lambda: w_copy(0, "u", bs[1]).start())
        def W(j):
            pltpu.make_async_copy(kv_s.at[slot, j], kv_s.at[slot, j], sem.at[slot * NB + j]).wait()
        def PX(j):
            b = bs[j]
            w_copy(0, "x", b, part).wait()
            for i, sl in enumerate((lo, hi)):
                qs = _quads(f(x_s[part, b, :, sl]) * c)
                for t, m in enumerate(_alpha(*[(lambda q=q: q) for q in qs])): xf[b, i, t] = m()
        def PT(j):
            b = bs[j]
            w_copy(0, "t", b, part).wait()
            for i, sl in enumerate((lo, hi)):
                for t, m in enumerate(_beta(f(wq_s[part, b, 1, sl, :]))): tf[b, i, t] = m
        def PS(j):
            b = bs[j]
            w_copy(0, "s", b, part).wait()
            for i, sl in enumerate((lo, hi)):
                w = f(wo_s[part, b, 1, :, sl])
                for t, m in enumerate(_beta(-w if i == 1 else w)): sf[b, i, t] = m
        def PU(j):
            g = bs[j]
            if first: w_copy(0, "u", g, part).wait()
            else: pl.when(a < NB - 1)(lambda: w_copy(0, "u", g, part).wait())
            for i, sl in enumerate((lo, hi)):
                for t, m in enumerate(_beta(f(wq_s[part, g, 0, sl, :]))): uf[g % 2, i, t] = m
        def PR(_):
            w_copy(0, "r", a, part).wait()
            for i, sl in enumerate((lo, hi)):
                w = f(wo_s[part, a, 0, :, sl])
                for t, m in enumerate(_beta(-w if i == 0 else w)): rf[a, i, t] = m
        ld = lambda name, ref, j, g, i, t: memo((name, j, i, t), lambda: ref[g, i, t])
        def MD(kind, j, t):
            g = bs[j]
            x = lambda i: ld("dx", xf, (kind // 2, j), g, i, t)
            w = lambda i: ld("dw", (tf, uf)[kind // 2], (kind // 2, j), (g, g % 2)[kind // 2], i, t)
            val["md", kind, j, t] = (lambda: _mm(x(0) + x(1), w(0)), lambda: _mm(x(1), w(1) - w(0)), lambda: _mm(x(0), w(0) - w(1)), lambda: _mm(x(0) + x(1), w(1)))[kind]()
            if all(("md", kind, j, u) in val for u in range(T)):
                for q, m in enumerate(_gamma([val["md", kind, j, u] for u in range(T)])):
                    if kind < 2: md_s[g, kind, q] = m
                    else: mu_s[g % 2, kind - 2, q] = m
        def M(kind, j, t):
            b = bs[j]
            tag = (j, kind if not cfg.share_m else 0)
            xa_ = lambda i: ld("xa", xf, tag, a, i, t); xb_ = lambda i: ld("xb", xf, tag, b, i, t)
            tb = lambda i: ld("tb", tf, tag, b, i, t); ua = lambda i: ld("ua", uf, tag, slot, i, t)
            if kind == 1: val["m1", j, t] = _mm(xa_(0) + xb_(1), tb(0) + ua(1))
            if kind == 7: val["z", j, 0, t] = val["m1", j, t] + _mm(xa_(1) - xb_(1), tb(1) + ua(1))
            if kind == 6: val["z", j, 1, t] = val["m1", j, t] + _mm(xb_(0) - xa_(0), tb(0) + ua(0))
        def query(j, i):
            k, col = divmod(i, 2); b = bs[j]
            if j == NB - 1:
                qs = [md_s[a, 0, q] + md_s[a, 1, q] if k == 0 else mu_s[slot, 0, q] + mu_s[slot, 1, q] for q in (col, 2 + col)]
            else:
                g = _gamma([val["z", j, k, t] for t in range(T)])
                qs = [g[q] + (md_s[b, 1, q] - mu_s[slot, 1, q] if k == 0 else mu_s[slot, 0, q] - md_s[b, 0, q]) for q in (col, 2 + col)]
            return h(jnp.concatenate(qs, axis=0))
        def tie(y, *xs):
            g = zero
            for x in xs: g = g & lax.bitcast_convert_type(x, I32)
            return lax.bitcast_convert_type(lax.bitcast_convert_type(y, I32) | g, F32)
        def S(j, i):
            s = lax.dot_general(query(j, i), kv_s[slot, j, i // 2, i % 2], (((1,), (1,)), ((), ())), preferred_element_type=F32)
            e = jnp.exp2(s - jnp.max(s, axis=-1, keepdims=True))
            ps = (e[:, :128] + e[:, 128:256]) + (e[:, 256:384] + e[:, 384:])
            l = jnp.sum(ps, axis=-1, keepdims=True)
            r = pltpu.reciprocal(l, approx=True)
            val["r", j, i] = r * (2.0 - l * r) if cfg.newton else r
            if cfg.glue:
                rows = []
                n = SQ // 16
                for ch in range(n):
                    y = e[16 * ch:16 * ch + 8, :128]
                    src = [u for u in range(n) if min(u + cfg.glue, n - 1) == ch]
                    if src: y = tie(y, *[ps[8 * v:8 * v + 8] for u in src for v in (2 * u, 2 * u + 1)])
                    rows += [y, e[16 * ch + 8:16 * ch + 16, :128]]
                e = jnp.concatenate([jnp.concatenate(rows, axis=0), e[:, 128:]], axis=1)
            val["p", j, i] = h(e)
        def V(j, i):
            val["o", j, i] = jnp.dot(val["p", j, i], kv_s[slot, j, 2 + i // 2, i % 2], preferred_element_type=F32) * val["r", j, i]
        def upd(ref, idx, v, init):
            ref[idx] = v if init else ref[idx] + v
        def G(j, i):
            b = bs[j]; o = val["o", j, i]; k, col = divmod(i, 2)
            if j == NB - 1:
                if k == 0: upd(gb_s, (0, a, col), -o, first); upd(gb_s, (1, a, col), o, first)
                else: upd(ga_s, (0, a, col), o, False); upd(ga_s, (1, a, col), -o, False)
            else:
                upd(gb_s, (1 - k, b, col), o, first); upd(ga_s, (1 - k, a, col), o, j == 0)
        def N(kind, j, t):
            b = bs[j]
            def al(k):
                o0, o1 = val["o", j, 2 * k], val["o", j, 2 * k + 1]
                return memo(("al", j, k, t), _alpha(lambda: o0[top], lambda: o1[top], lambda: o0[bot], lambda: o1[bot])[t])
            sb = lambda i: ld("sb", sf, j, b, i, t); ra = lambda i: ld("ra", rf, j, a, i, t)
            if kind == 1: val["n1", j, t] = _mm(al(0) + al(1), sb(0) + ra(1))
            if kind == 7:
                n = _mm(al(0), sb(1) - ra(1))
                upd(accb, (b, 1, t), val["n1", j, t] + n, first); upd(acca, (a, 1, t), n, j == 0)
            if kind == 6:
                n = _mm(al(1), ra(0) - sb(0))
                upd(accb, (b, 0, t), n, first); upd(acca, (a, 0, t), val["n1", j, t] + n, j == 0)
        def Z(_):
            for i in range(2):
                for t in range(T): accb[a, i, t] = jnp.zeros((HR, 128), F32)
        fn = dict(D=D, W=W, PX=PX, PT=PT, PS=PS, PU=PU, PR=PR, MD=MD, M=M, S=S, V=V, G=G, N=N, Z=Z)
        for op, *args in order:
            fn[op](*args)

    for j in range(cfg.ahead):
        start_first(j)

    def part_body(part, _):
        if not cfg.only_l: iteration(part, 0, True, cfg.order(True))
        def body(a, _):
            iteration(part, a, False, cfg.order(False))
            return 0
        lax.fori_loop(1, NB, body, 0)
        if cfg.only_l: return 0
        for b in range(NB):
            al = lambda ref, k: _alpha(lambda: ref[k, b, 0, top], lambda: ref[k, b, 1, top], lambda: ref[k, b, 0, bot], lambda: ref[k, b, 1, bot])
            g2n, g4, g3, g5n = al(gb_s, 0), al(gb_s, 1), al(ga_s, 0), al(ga_s, 1)
            z1, z2 = [], []
            for t in range(T):
                s1, s2n, r1n, r2 = sf[b, 0, t], sf[b, 1, t], rf[b, 0, t], rf[b, 1, t]
                n25 = _mm(g2n[t](), s1) + _mm(g5n[t](), r2)
                z1.append((accb[b, 0, t] - acca[b, 0, t]) + n25 + _mm(g3[t](), r1n + r2))
                z2.append((acca[b, 1, t] - accb[b, 1, t]) + n25 + _mm(g4[t](), s2n + s1))
            for i, z in enumerate((z1, z2)):
                for q, m in enumerate(_gamma(z)):
                    ob_s[part, b, (top, bot)[q // 2], pl.ds(i * HW + (q % 2) * 128, 128)] = h(-m)
            out_copy(part, b).start()
        return 0

    lax.fori_loop(0, 2, part_body, 0)
    if cfg.only_l: return
    for p in range(2):
        for b in range(NB):
            out_copy(p, b).wait()

TORD = (0, 6, 3, 4, 1, 2, 5)
def order_a(first):
    L = NB - 1
    M = lambda k, j: [("M", k, j, t) for t in TORD]
    M76 = lambda j: [("M", k, j, t) for t in TORD for k in (7, 6)]
    MD = lambda k, j: [("MD", kk, j, t) for t in TORD for kk in k]
    rounds = lambda ps: [ps[i:i + 4] for i in range(0, len(ps), 4)]
    nxt = MD((2, 3), 0)
    o = []
    if first:
        o += [("Z", 0), ("PX", L), ("PU", L)] + MD((2, 3), L) + [("PX", 0), ("PT", 0)] + MD((0, 1), 0)
        pre = M(1, 0) + M(7, 0) + M(6, 0)
        o += pre[:20]; carry = pre[20:]
    else:
        pre = M(1, 0) + M(7, 0) + M(6, 0)
        o += pre[:20]; carry = pre[20:]
    for j in range(NB):
        ps = list(carry); carry = []
        m1 = M(1, j + 1) if j + 1 < L else []
        if j > 0:
            fill = ps + m1
            if not m1:
                fill += nxt[:7]; nxt = nxt[7:]
            ps = []
            for t in range(T):
                ps += [("N", 1, j - 1, t), ("N", 7, j - 1, t), ("N", 6, j - 1, t)] + fill[:1]; fill = fill[1:]
            ps += fill
        else:
            ps += m1
        if first and j + 1 < L: ps += MD((0, 1), j + 1)
        if first and j + 1 == L: ps = MD((0, 1), j + 1)[:12] + ps[:4] + MD((0, 1), j + 1)[12:] + ps[4:]
        if j + 1 < L: ps += M(7, j + 1) + M(6, j + 1)
        k = len(ps) // 4 * 4 if j < L else len(ps)
        ps, carry = ps[:k], ps[k:]
        rs = rounds(ps)
        n = len(rs)
        cut = [(n * s + 7) // 8 for s in range(9)]
        o += [("D", j), ("W", j)]
        if first and j < L:
            if j + 1 < L: o += [("PX", j + 1)]
            o += [("PT", j + 1)]
        if first and j > 0: o += [("PS", j - 1)]
        if j == 1: o += [("PR", 0)]
        if j == L - 1: o += [("PU", 0)]
        for s in range(8):
            o += [("SV"[s % 2], j, s // 2)]
            if s % 2: o += [("G", j, s // 2)]
            for r in rs[cut[s]:cut[s + 1]]: o += r
    if first: o += [("PS", L)]
    return o

def make(name, flags=None, **kw):
    kw.setdefault("order", order_a); kw.setdefault("share_m", False)
    cfg = Cfg(**kw)
    flags = dict({"XLA_TPU_RESCHEDULE_DMA_DONES": True}, **(flags or {}))
    def fn(A_x, A_k, A_v, A_wq, A_wo, B_x, B_k, B_v, B_wq, B_wo):
        B, SQ, D = A_x.shape
        _, H, SK, DH = A_k.shape
        rs = lambda t: t.reshape(B, NB, 2, 2, SK, DH)
        act, wgt = (SQ // 2, DH), (DH, DH)
        return pl.pallas_call(
            functools.partial(_kernel, cfg=cfg),
            in_specs=[pl.BlockSpec(memory_space=pl.ANY)] * 10,
            out_specs=pl.BlockSpec(memory_space=pl.ANY),
            out_shape=jax.ShapeDtypeStruct((B, SQ, 2 * D), A_x.dtype),
            scratch_shapes=[
                pltpu.VMEM((2, B, SQ, D), BF16), pltpu.VMEM((2, NB, 2, D, HW), BF16), pltpu.VMEM((2, NB, 2, HW, D), BF16),
                pltpu.VMEM((2, NB, 4, 2, SK, DH), BF16),
                pltpu.VMEM((NB, 2, T) + act, F32), pltpu.VMEM((NB, 2, T) + wgt, F32), pltpu.VMEM((NB, 2, T) + wgt, F32),
                pltpu.VMEM((2, 2, T) + wgt, F32), pltpu.VMEM((NB, 2, T) + wgt, F32),
                pltpu.VMEM((NB, 2, 4) + act, F32), pltpu.VMEM((2, 2, 4) + act, F32),
                pltpu.VMEM((2, NB, 2, SQ, DH), F32), pltpu.VMEM((2, NB, 2, SQ, DH), F32),
                pltpu.VMEM((NB, 2, T) + act, F32), pltpu.VMEM((NB, 2, T) + act, F32), pltpu.VMEM((2, B, SQ, D), BF16),
                pltpu.SemaphoreType.DMA((12 * NB,)), pltpu.SemaphoreType.DMA((2, NB)),
            ],
            compiler_params=pltpu.CompilerParams(vmem_limit_bytes=120 * 1024 * 1024, flags=flags, disable_bounds_checks=True),
            name=name,
        )(A_x, rs(A_k), rs(A_v), A_wq, A_wo, B_x, rs(B_k), rs(B_v), B_wq, B_wo)
    return fn


@jax.jit
def pallas_concat_heads__gqa_block_cached__mha_block_cached__near_ridge_kernel(
    A_x, A_k_cache, A_v_cache, A_wq, A_wo, B_x, B_k_cache, B_v_cache, B_wq, B_wo):
    return make("attn_blocks", glue=1)(A_x, A_k_cache, A_v_cache, A_wq, A_wo, B_x, B_k_cache, B_v_cache, B_wq, B_wo)
```

```python
import functools

import jax
import jax.numpy as jnp
from jax import lax
import jax.experimental.pallas as pl
import jax.experimental.pallas.tpu as pltpu

F32, BF16, I32 = jnp.float32, jnp.bfloat16, jnp.int32
LOG2E = 1.4426950408889634
NB = 8
NH = 4 * NB
DH = 128
HW = 2 * DH
T = 7
AHEAD = 12
M_ORDER = (0, 6, 3, 4, 1, 2, 5)
EARLY = (("x", 0), ("t", 0), ("x", 1), ("t", 1))

TUNING = dict(
    first=dict(
        n_order=(3, 4, 5, 2, 6, 0, 1), paired=(2, 3, 5, 6, 7), gate=64,
        plan=(
            "*m3 m3 m3 m3 S7 m1 V3 m2 m4 176", "*S7 m1 V2 m2 m2 m 176",
            "*S5 m2 V m 192", "S6 m2 V2 m m2 m 176",
            "*S6 m2 V3 m 176", "*S6 m1 V3 m2 192",
            "*S6 N1 V N 176", "*S N V N m m m 176",
            "*S7 N1 V2 N1 m3 m3 m 192", "*S7 N1 V3 m2 192",
            "*S7 N1 V3 N2 m2 m1 176", "*S N V N m m N m 160",
            "*S6 N1 V3 N2 192", "*S8 m V3 N2 m2 176",
            "*S6 N1 V3 m2 176", "*S6 N V N1 m m 176",
            "*S7 N1 V3 n2 m2 m2 m2 176", "*S6 N V2 m2 192",
            "*S7 N2 V3 N5 176", "*S m V N N m m m m 176",
            "*S8 N1 V3 m2 176", "*S6 N1 V3 N1 m2 m 176",
            "*S8 N1 V3 N4 176", "*S3 n V N m m m 176",
            "*S7 N1 V3 m2 N2 N1 m 176", "*S m V 224",
            "*S6 m V2 n 176", "*S8 N V m N 176",
            "*S7 N V2 m 192", "*S6 N V 176",
            "*S5 N V2 N1 N N N 176", "*S8 N V1 192",
        ),
    ),
    rest=dict(
        n_order=(3, 5, 2, 4, 0, 1, 6), paired=(2, 5, 6, 7), gate=0,
        plan=(
            "*m S m V m 160", "*S m V m1 m m 176", "*S m1 V1 192", "S7 m V m2 224",
            "*S m1 V1 192", "S1 m V1 176", "*S n V n m m 192", "S n V m n n 192",
            "*S n V m 224", "S N V 176", "S n V n 176", "S n V m n n 192",
            "*S n V m 176", "S n V m m 176", "S n V n n 176", "*S n V 176",
            "*S n V m n m 224", "S n V 224", "S n V n m 176", "S n V m 192",
            "S N V m n m n 192", "S n V m 208", "*S n V n 176", "S n V m n 192",
            "S n V 176", "S N V m m n 208", "S n V m N 208", "S n V 176",
            "S7 n V1 176", "S6 n1 V 192", "*S N V1 n N 208", "S n V N n 192",
        ),
    ),
)


def _dot(a, b):
    return jnp.dot(a.astype(BF16), b.astype(BF16), preferred_element_type=F32)


def _lhs_term(quad, t):
    i, j, sub = ((0, 3, 0), (2, 3, 0), (0, None, 0), (3, None, 0), (0, 1, 0), (2, 0, 1), (1, 3, 1))[t]
    return quad(i) if j is None else quad(i) - quad(j) if sub else quad(i) + quad(j)


def _rhs_term(quad, t):
    i, j, sub = ((0, 3, 0), (0, None, 0), (1, 3, 1), (2, 0, 1), (3, None, 0), (0, 1, 0), (2, 3, 0))[t]
    return quad(i) if j is None else quad(i) - quad(j) if sub else quad(i) + quad(j)


def _result_quad(m, q):
    if q == 0:
        return (m(0) + m(6)) + (m(3) - m(4))
    if q == 3:
        return (m(0) + m(5)) + (m(2) - m(1))
    return m(2) + m(4) if q == 1 else m(1) + m(3)


def _signed(y, n, scale=1.0):
    if not isinstance(n, int):
        return y * jnp.where(n & 1 == 1, -scale, scale).astype(F32)
    if scale != 1.0:
        return y * (-scale if n % 2 else scale)
    return -y if n % 2 else y


def _after(zero, y, *xs):
    for x in xs:
        zero = zero & lax.bitcast_convert_type(x, I32)
    zero = jnp.concatenate([zero] * (y.shape[0] // 8), axis=0)
    return lax.bitcast_convert_type(lax.bitcast_convert_type(y, I32) | zero, F32)


def _aligned(i, n):
    return i if isinstance(i, int) else pl.multiple_of(i, n)


def _chunks(name):
    return 14 if name == "x" else 16


def _head(hd):
    unit, col = divmod(hd, 2)
    side = 0 if unit == 0 else 1 if unit == 2 * NB - 1 else (unit + 1) % 2
    return (unit + 1) // 2 % NB, side, col


def _program(first, tune):
    pair = lambda kinds, j: [("M", k, j, t) for t in M_ORDER for k in kinds]
    shared = lambda k, j: [("D", k, j, t) for t in M_ORDER if first or k in (3, 5)]
    ms = shared(2, 0) + shared(4, 0)
    for j in range(1, NB):
        ms += (shared(5, 0) if j == 1 else []) + shared(4, j)
        ms += pair((1, 7), j) if j in tune["paired"] else pair((1,), j) + pair((7,), j)
        ms += (shared(3, 0) if j == 1 else []) + shared(2, j) + pair((6,), j)
    operands = [("r", 0)]
    if first:
        operands = [("x", 2), ("t", 2), ("s", 1), ("r", 0)]
        for j in range(3, NB):
            operands += [("x", j), ("t", j), ("s", j - 1)]
        operands += [("s", NB - 1)]
    queue = [(name, j, ch) for name, j in operands for ch in range(_chunks(name))]
    ns, ops, fetch, waits = [], [], {}, []
    for hd, line in enumerate(tune["plan"]):
        *slots, due = line.lstrip("*").split()
        if line[0] == "*":
            waits.append(hd)
        if hd % 4 == 2 and hd > 2:
            ns += [("N", k, hd // 4, t) for t in tune["n_order"] for k in (1, 7, 6)]
        if hd == NH - 4:
            queue += [(name, j, ch) for name, j in [("u", 1), ("s", 0)][:1 + first] for ch in range(16)]
        dma = [("DMA", hd)]
        for slot in slots:
            kind, count = slot[0], int(slot[1:] or 0)
            if count or kind == "S":
                ops, dma = ops + dma, []
            for n in range(count):
                name, j, ch = queue.pop(0)
                if ch == 0:
                    fetch.setdefault(hd, []).append((name, j))
                ops.append(("P", name, j, ch, (224 if kind in "SV" else 112) * n // count))
            if kind in "SV":
                ops.append((kind, hd, int(due)))
                continue
            tiles = [ns.pop(0) for _ in range(min(3, len(ns)) if kind in "nN" else 0)]
            while len(tiles) < 4:
                tiles.append((ms or ns).pop(0))
            for op, _, j, _ in tiles:
                uses = (("s", j), ("r", 0)) if op == "N" else (("x", j), ("t", j))
                assert not any(item[:2] in uses for item in queue)
            ops += sorted(tiles, key=lambda tile: tile[0] == "N") if kind.isupper() else tiles
    assert len(tune["plan"]) == NH and waits[0] == 0 and not (ms or ns or queue)
    owner = [max(w for w in waits if w <= hd) for hd in range(NH)]
    assert all(hd - w < AHEAD for hd, w in enumerate(owner))
    return ops, fetch, owner


def _kernel(xa, ka, va, wqa, woa, xb, kb, vb, wqb, wob, out,
            x_raw, wq_raw, wo_raw, kv, xf, tf, sf, uf, rf, m24, acc_b, acc_a, out_buf,
            sem, out_sem):
    hbm = ((xa, ka, va, wqa, woa), (xb, kb, vb, wqb, wob))
    sq = x_raw.shape[1]
    hr = sq // 2
    halves = (slice(0, hr), slice(hr, sq))
    scale = DH ** -0.5 * LOG2E
    programs = {True: _program(True, TUNING["first"]), False: _program(False, TUNING["rest"])}
    wrap = lambda g: g & (NB - 1)

    def operand_copy(p, name, g, s):
        x, _, _, wq, wo = hbm[p]
        if name == "x":
            return pltpu.make_async_copy(x.at[g], x_raw.at[g], s)
        heads = pl.ds(_aligned(g * 2 * HW, 2 * HW) + (HW if name in "ts" else 0), HW)
        slot = g if name in "ts" else NB
        if name in "ut":
            return pltpu.make_async_copy(wq.at[:, heads], wq_raw.at[slot], s)
        return pltpu.make_async_copy(wo.at[heads, :], wo_raw.at[slot], s)

    def head_copies(p, a, hd, first, skip=""):
        _, fetch, owner = programs[first]
        j, side, col = _head(hd)
        b = wrap(a + j)
        s = sem.at[owner[hd]]
        copies = [operand_copy(p, name, wrap(a + g), s) for name, g in fetch.get(hd, ()) if name != skip]
        for n, src in enumerate(hbm[p][1:3]):
            src = src.at[a, 4 * b + 2 + col] if side == 0 else src.at[b, 4 * a + col]
            copies.append(pltpu.make_async_copy(src, kv.at[hd, n], s))
        return copies

    def start_head(p, a, hd, first):
        for copy in head_copies(p, a, hd, first, skip="u"):
            copy.start()

    def out_copy(part, b):
        cols = pl.ds(_aligned(part * 2 * HW, 2 * HW), 2 * HW)
        return pltpu.make_async_copy(out_buf.at[part, b], out.at[b, :, cols], out_sem.at[part])

    def prepare(name, g, i, r, gate=lambda y: y):
        slot = NB if name in "ur" else g
        tile = lambda n: pl.ds(_aligned(n * DH, DH), DH)
        rows = lambda o: pl.ds(_aligned(o + 16 * r, 16), 16)
        quads = []
        for q in range(4):
            if name == "x":
                y = _signed(x_raw[slot, rows(q // 2 * hr), tile(2 * i + q % 2)].astype(F32), i + q % 2, scale)
            elif name in "ut":
                y = _signed(wq_raw[slot, rows((2 * i + q // 2) * DH), tile(q % 2)].astype(F32), i + q // 2)
            else:
                y = _signed(wo_raw[slot, rows(q // 2 * DH), tile(2 * i + q % 2)].astype(F32), g + (i + q // 2))
            quads.append(gate(y))
        dst = uf.at[g & 1] if name == "u" else dict(x=xf, t=tf, s=sf, r=rf)[name].at[g]
        terms = [(_lhs_term if name == "x" else _rhs_term)(lambda q: quads[q], t) for t in range(T)]
        for t, y in enumerate(terms):
            dst[i, t, pl.ds(16 * r, 16)] = y
        return terms

    def iteration(part, a, first):
        ops, fetch, owner = programs[first]
        gate_lead = TUNING["first" if first else "rest"]["gate"]
        partner = [wrap(a + j) for j in range(NB)]
        after = functools.partial(_after, jnp.full((8, DH), part >> 1, I32))
        val, due, produced, clock = {}, [], [], [0]
        now = lambda: clock[0] // hr * hr

        def once(key, fn):
            if key not in val:
                val[key] = fn()
            return val[key]

        def needed_by(y, time):
            due.extend((time + r // 16 * 16, y[r:r + 8]) for r in range(0, y.shape[0], 8))

        def ready_at(y, time):
            produced.extend((time + r, y, r) for r in range(0, y.shape[0], 16))

        def paced(y):
            if not due:
                return y
            pieces = []
            for r in range(0, y.shape[0], 16):
                xs = [x for time, x in due if time <= now() + r]
                due[:] = [(time, x) for time, x in due if time > now() + r]
                pieces += [after(y[r:r + 8], *xs) if xs else y[r:r + 8], y[r + 8:r + 16]]
            return jnp.concatenate(pieces, axis=0)

        def tile(x, w):
            y = _dot(paced(x), w)
            if clock[0] % hr == 0:
                ready_at(y, clock[0] + 130)
            clock[0] += hr // 4
            return y

        def add_to(ref, idx, y, init):
            y = y if init else ref[idx] + y
            ref[idx] = y
            return y

        def dma(hd):
            t = hd + AHEAD
            last = a == NB - 1
            if t < NH:
                for p in range(2):
                    pl.when(part == p)(lambda: start_head(p, a, t, first))
                if ("u", 1) in fetch.get(t, ()):
                    nxt = part + ((a + 1) >> 3)
                    pl.when(nxt == 0)(lambda: operand_copy(0, "u", partner[1], sem.at[owner[t]]).start())
                    pl.when(nxt > 0)(lambda: operand_copy(1, "u", partner[1], sem.at[owner[t]]).start())
            else:
                for p in range(2):
                    pl.when(jnp.logical_and(part == p, a < NB - 1))(
                        lambda: start_head(p, partner[1], t - NH, False))
                if not first:
                    pl.when(jnp.logical_and(part == 0, last))(lambda: start_head(1, 0, t - NH, True))
            if not first and 2 <= hd < 2 + len(EARLY):
                pl.when(jnp.logical_and(part == 0, a == NB - 2))(
                    lambda: operand_copy(1, *EARLY[hd - 2], sem.at[NH]).start())
            for w in range(NH):
                if owner[w] == hd:
                    for copy in head_copies(0, a, w, first):
                        copy.wait()

        def prepare_chunk(name, j, ch, dt):
            gate = lambda y: y
            past = [item for item in produced if gate_lead and item[0] <= clock[0] + dt - gate_lead]
            if past:
                _, src, r = max(past, key=lambda item: item[0])
                gate = lambda y: after(y, src[r:r + 8, :DH])
            needed_by(prepare(name, partner[j], ch % 2, ch // 2, gate)[0], clock[0] + dt)

        def shared_product(kind, j, t):
            g = partner[j]
            x = lambda i: xf[g, i, t]
            w = lambda i: tf[g, i, t] if kind in (2, 4) else uf[a & 1, i, t]
            if kind in (2, 5):
                val["d", kind, j, t] = tile(x(0) + x(1), w(0 if kind == 2 else 1))
            else:
                val["d", kind, j, t] = tile(x(1), w(1) - w(0)) if kind == 4 else tile(x(0), w(0) - w(1))
            if t == M_ORDER[-1]:
                for q in range(4):
                    val["dq", kind, j, q] = _result_quad(lambda s: val["d", kind, j, s], q)
                    if kind in (2, 4):
                        m24[g, kind // 2 - 1, q] = val["dq", kind, j, q]

        def query_product(kind, j, t):
            b = partner[j]
            load = lambda name, ref, g, i: once((name, j, now(), i, t), lambda: ref[g, i, t])
            x_a, x_b = (lambda i: load("xa", xf, a, i)), (lambda i: load("xb", xf, b, i))
            t_b, u_a = (lambda i: load("tb", tf, b, i)), (lambda i: load("ua", uf, a & 1, i))
            if kind == 1:
                val["m1", j, t] = tile(x_a(0) + x_b(1), t_b(0) + u_a(1))
            elif kind == 7:
                val["z", j, 0, t] = val["m1", j, t] + tile(x_a(1) - x_b(1), t_b(1) + u_a(1))
            else:
                val["z", j, 1, t] = val["m1", j, t] + tile(x_b(0) - x_a(0), t_b(0) + u_a(0))

        def scores(hd, _):
            j, side, col = _head(hd)
            assert not first or ("dq", (4, 2)[side], j, 0) in val
            m = lambda k, q: val["dq", k, 0, q] if k in (3, 5) else m24[partner[j], k // 2 - 1, q]
            if j == 0:
                rows = [m(2 + side, q) + m(4 + side, q) for q in (col, 2 + col)]
            else:
                rows = [_result_quad(lambda t: val["z", j, side, t], q)
                        + (m(4, q) - m(5, q) if side == 0 else m(3, q) - m(2, q)) for q in (col, 2 + col)]
            query = paced(jnp.concatenate(rows, axis=0)).astype(BF16)
            val["s", hd] = lax.dot_general(query, kv[hd, 0], (((1,), (1,)), ((), ())),
                                           preferred_element_type=F32)
            ready_at(val["s", hd], clock[0] + 130)
            clock[0] += sq

        def attend(hd, settle):
            j, side, col = _head(hd)
            s = val["s", hd]
            e = jnp.exp2(s - jnp.max(s, axis=-1, keepdims=True))
            total = (e[:, :DH] + e[:, DH:2 * DH]) + (e[:, 2 * DH:3 * DH] + e[:, 3 * DH:])
            inv = pltpu.reciprocal(jnp.sum(total, axis=-1, keepdims=True), approx=True)
            p = jnp.concatenate([paced(e[:, :DH]), e[:, DH:]], axis=1)
            o = _dot(p, kv[hd, 1]) * _signed(inv, j + side + col)
            ready_at(o, clock[0] + 150)
            for n, half in enumerate(halves):
                q = 2 * n + col
                val["o", j, side, q] = y = o[half]
                if j:
                    sums = [add_to(acc_b, (partner[j], 1 - side, T + q), y, first),
                            add_to(acc_a, (a, 1 - side, T + q), y, j == 1)]
                elif side == 0:
                    sums = [add_to(acc_b, (a, 0, T + q), -y, first), add_to(acc_b, (a, 1, T + q), y, first)]
                else:
                    sums = [add_to(acc_a, (a, 0, T + q), y, False), add_to(acc_a, (a, 1, T + q), -y, False)]
                for z in sums:
                    needed_by(z, clock[0] + n * hr + settle)
            clock[0] += sq

        def out_product(kind, j, t):
            b = partner[j]
            o = lambda side: once(("o'", j, side, t), lambda: _lhs_term(lambda q: val["o", j, side, q], t))
            load = lambda name, ref, g, i: once((name, j, now(), i, t), lambda: ref[g, i, t])
            s_b, r_a = (lambda i: load("sb", sf, b, i)), (lambda i: load("ra", rf, a, i))
            if kind == 1:
                val["n1", j, t] = tile(o(0) + o(1), s_b(0) + r_a(1))
            elif kind == 7:
                y = tile(o(0), s_b(1) - r_a(1))
                add_to(acc_b, (b, 1, t), val["n1", j, t] + y, first)
                add_to(acc_a, (a, 1, t), y, j == 1)
            else:
                y = tile(o(1), r_a(0) - s_b(0))
                add_to(acc_b, (b, 0, t), y, first)
                add_to(acc_a, (a, 0, t), val["n1", j, t] + y, j == 1)

        run = dict(DMA=dma, P=prepare_chunk, D=shared_product, M=query_product, S=scores, V=attend,
                   N=out_product)
        for op, *args in ops:
            run[op](*args)

    def finish(part):
        @pl.when(part == 0)
        def _():
            for name, g in EARLY:
                operand_copy(1, name, g, sem.at[NH]).wait()

        todo = [(name, g, ch % 2, ch // 2) for name, g in EARLY for ch in range(_chunks(name))]
        after = functools.partial(_after, jnp.full((8, DH), part >> 1, I32))
        for b in range(NB):
            lhs = lambda ref, k, t: _lhs_term(lambda q: ref[b, k, T + q], t)
            z = {}
            for n, t in enumerate(M_ORDER, b * T):
                s1, s2, r1, r2 = sf[b, 0, t], sf[b, 1, t], rf[b, 0, t], rf[b, 1, t]
                y = lhs(acc_b, 0, t)
                for item in todo[len(todo) * n // (NB * T):len(todo) * (n + 1) // (NB * T)]:
                    x = prepare(*item)[0]
                    y = jnp.concatenate([y[:48], after(y[48:56], x[:8], x[8:]), y[56:]], axis=0)
                both = _dot(y, s1) + _dot(lhs(acc_a, 1, t), r2)
                z[0, t] = (acc_b[b, 0, t] - acc_a[b, 0, t]) + both + _dot(lhs(acc_a, 0, t), r1 + r2)
                z[1, t] = (acc_a[b, 1, t] - acc_b[b, 1, t]) + both + _dot(lhs(acc_b, 1, t), s2 + s1)
                if b == 0:
                    for i in range(2):
                        acc_b[0, i, t] = jnp.zeros((hr, DH), F32)
            for i in range(2):
                for q in range(4):
                    y = _signed(_result_quad(lambda t: z[i, t], q), b + 1)
                    out_buf[part, b, halves[q // 2], pl.ds(i * HW + q % 2 * DH, DH)] = y.astype(out_buf.dtype)
            out_copy(part, b).start()

    warmup = (("u", 0),) + EARLY
    for n, (name, g) in enumerate(warmup):
        operand_copy(0, name, g, sem.at[NH + 1 + n]).start()
    for hd in range(AHEAD):
        start_head(0, 0, hd, True)
    for i in range(2):
        for t in range(T):
            acc_b[0, i, t] = jnp.zeros((hr, DH), F32)
    for n, (name, g) in enumerate(warmup):
        operand_copy(0, name, g, sem.at[NH + 1 + n]).wait()

        def half(i, carry):
            for r in range(_chunks(name) // 2):
                prepare(name, g, i, r)
            return carry

        lax.fori_loop(0, 2, half, 0)

    def block(part, carry):
        def rest(a, inner):
            iteration(part, a, False)
            return inner

        iteration(part, 0, True)
        lax.fori_loop(1, NB, rest, 0)
        finish(part)
        return carry

    lax.fori_loop(0, 2, block, 0)
    for p in range(2):
        for b in range(NB):
            out_copy(p, b).wait()


@jax.jit
def pallas_concat_heads__gqa_block_cached__mha_block_cached__near_ridge_kernel(
    A_x: jax.Array,
    A_k_cache: jax.Array,
    A_v_cache: jax.Array,
    A_wq: jax.Array,
    A_wo: jax.Array,
    B_x: jax.Array,
    B_k_cache: jax.Array,
    B_v_cache: jax.Array,
    B_wq: jax.Array,
    B_wo: jax.Array,
):
    batch, sq, d = A_x.shape
    sk = A_k_cache.shape[2]
    assert (batch, sq, d) == (NB, 224, 2 * HW) and A_k_cache.shape == (NB, NH, 4 * DH, DH)
    rows, tile = (sq // 2, DH), (DH, DH)
    return pl.pallas_call(
        _kernel,
        in_specs=[pl.BlockSpec(memory_space=pl.ANY)] * 10,
        out_specs=pl.BlockSpec(memory_space=pl.ANY),
        out_shape=jax.ShapeDtypeStruct((batch, sq, 2 * d), A_x.dtype),
        scratch_shapes=[
            pltpu.VMEM((NB, sq, d), BF16),
            pltpu.VMEM((NB + 1, d, HW), BF16),
            pltpu.VMEM((NB + 1, HW, d), BF16),
            pltpu.VMEM((NH, 2, sk, DH), BF16),
            pltpu.VMEM((NB, 2, T) + rows, F32),
            pltpu.VMEM((NB, 2, T) + tile, F32),
            pltpu.VMEM((NB, 2, T) + tile, F32),
            pltpu.VMEM((2, 2, T) + tile, F32),
            pltpu.VMEM((NB, 2, T) + tile, F32),
            pltpu.VMEM((NB, 2, 4) + rows, F32),
            pltpu.VMEM((NB, 2, T + 4) + rows, F32),
            pltpu.VMEM((NB, 2, T + 4) + rows, F32),
            pltpu.VMEM((2, NB, sq, d), A_x.dtype),
            pltpu.SemaphoreType.DMA((NH + 2 + len(EARLY),)),
            pltpu.SemaphoreType.DMA((2,)),
        ],
        compiler_params=pltpu.CompilerParams(
            vmem_limit_bytes=110 * 1024 * 1024,
            flags={"XLA_TPU_RESCHEDULE_DMA_DONES": True},
            disable_bounds_checks=True,
            disable_semaphore_checks=True,
        ),
        name="attn_blocks",
    )(A_x, A_k_cache, A_v_cache, A_wq, A_wo, B_x, B_k_cache, B_v_cache, B_wq, B_wo)
```
